```python
import os as _os
_os.environ.setdefault("JAX_PLATFORMS", "cpu")
import jax
import jax.numpy as jnp

def _softmax(x, axis=-1):
    return jax.nn.softmax(x, axis=axis)
def _gelu(x):
    return jax.nn.gelu(x, approximate=True)
def _silu(x):
    return jax.nn.silu(x)
def _sigmoid(x):
    return jax.nn.sigmoid(x)
def _layernorm(x, axis=-1, eps=1e-5):
    m = jnp.mean(x, axis=axis, keepdims=True)
    v = jnp.var(x, axis=axis, keepdims=True)
    return (x - m) / jnp.sqrt(v + eps)
def _scatter_add(tgt, idx, src, axis=0):
    return tgt.at[idx].add(src)
def _segment_sum(src, seg, n):
    return jax.ops.segment_sum(src, seg, n)
class _Rng:
    def __init__(self, key):
        self._k = key
    def _next(self):
        self._k, sub = jax.random.split(self._k)
        return sub
    def normal(self, shape):
        return jax.random.normal(self._next(), shape, dtype=jnp.bfloat16)
    def randint(self, lo, hi, shape):
        return jax.random.randint(self._next(), shape, lo, hi, dtype=jnp.int32)
    def uniform(self, shape, lo=0.0, hi=1.0):
        return jax.random.uniform(self._next(), shape, jnp.bfloat16, lo, hi)
    def permutation(self, n):
        return jax.random.permutation(self._next(), n)


kernel_name = 'gated_mix__linear_attn_block__swiglu_ffn__prompt'

def setup_inputs():
    _rng = _Rng(jax.random.key(int.from_bytes(__import__("os").urandom(4), "little")))
    _w = (lambda a: (lambda t: t.astype(jnp.bfloat16) if jnp.issubdtype(t.dtype, jnp.floating) else t)(jnp.asarray(a)))
    def _A_setup():
        B, S, D = 1, 2048, 512
        return {
            "x": _w((lambda *s: _rng.normal(s) * 0.05)(B, S, D)),
            "wqkv": _w((lambda *s: _rng.normal(s) * 0.8)(D, 3 * D)),
            "wo": _w((lambda *s: _rng.normal(s) * 0.05)(D, D)),
        }
    _A_in = _A_setup()

    def _B_setup():
        B, S, D, F = 1, 2048, 512, 1792
        return {
            "x": _w((lambda *s: _rng.normal(s) * 0.05)(B, S, D)),
            "w_gate": _w((lambda *s: _rng.normal(s) * 0.1)(D, F)),
            "w_up": _w((lambda *s: _rng.normal(s) * 0.1)(D, F)),
            "w_down": _w((lambda *s: _rng.normal(s) * 0.1)(F, D)),
        }
    _B_in = _B_setup()

    return {
        "A_x": _A_in["x"],
        "A_wqkv": _A_in["wqkv"],
        "A_wo": _A_in["wo"],
        "B_x": _B_in["x"],
        "B_w_gate": _B_in["w_gate"],
        "B_w_up": _B_in["w_up"],
        "B_w_down": _B_in["w_down"],
        "gate_w": _w((lambda *s: _rng.normal(s) * 0.05)(512) * 16.0),
    }

def reference(A_x, A_wqkv, A_wo, B_x, B_w_gate, B_w_up, B_w_down, gate_w):
    def _A_ref(x, wqkv, wo):
        B, S, D = x.shape
        H = 32; Dh = D // H
        qkv = (lambda x, *d: x.transpose(*d))((x @ wqkv).reshape(B, S, 3, H, Dh), 2, 0, 3, 1, 4)
        q, k, v = qkv[0], qkv[1], qkv[2]
        phi = lambda t: jnp.where(t > 0, t + 1, jnp.exp(t)) + 1e-6
        pq, pk = phi(q), phi(k)
        kv = jnp.einsum("bhsd,bhse->bhde", pk, v)
        z = jnp.einsum("bhsd->bhd", pk)
        num = jnp.einsum("bhqd,bhde->bhqe", pq, kv)
        den = jnp.einsum("bhqd,bhd->bhq", pq, z)[..., None] + 1e-6
        o = num / den
        return (lambda x, *d: x.transpose(*d))(o, 0, 2, 1, 3).reshape(B, S, D) @ wo

    def _B_ref(x, w_gate, w_up, w_down):
        g = _silu(x @ w_gate)
        u = x @ w_up
        return (g * u) @ w_down

    x = A_x
    g = _sigmoid((x * gate_w).sum(-1, keepdims=True))
    a = _A_ref(x, A_wqkv, A_wo)
    b = _B_ref(x, B_w_gate, B_w_up, B_w_down)
    return g * a + (1 - g) * b
```

```python
import functools
import math
import jax
import jax.numpy as jnp
from jax import lax
import jax.experimental.pallas as pl
import jax.experimental.pallas.tpu as pltpu

N_HEADS = 32
H_DIM = 16
XSPLIT = (0, 128, 256, 1024, 2048)
SUB1 = 256
TM = 512
FC = 896
QPRE = 512
ORS = 128
UNR = 2
NOBC = True
QPOS = 1
APOS = 2
SILU = 0
GPOS = 1
GSPLIT = 0
GSPLIT2 = 1024
QEARLY = 0
QEARLY_POS = 2

f32 = jnp.float32
bf16 = jnp.bfloat16
u32 = jnp.uint32
NT = (((1,), (1,)), ((), ()))
LOG2E = 1.4426950408889634


def _phi(t):
    return jnp.where(t > 0, t + 1.0, jnp.exp(t)) + 1e-6


def _sigmoid(t):
    return pl.reciprocal(1.0 + jnp.exp2(t * (-LOG2E)), approx=True)


def _kernel(x_hbm, wqkv_hbm, wo_hbm, wg_hbm, wu_hbm, wd_hbm, gw_hbm, o_hbm,
            x_v, wq_v, wk_v, wv_v, wo_v, wg_v, wu_v, wd_v, gw_v, o_v,
            wkt_v, wqt_v, wqp_v, p_v, z_v, zp_v, zrow_v, kv_v, mp_v, pq_v, g_v, sem, *, S, D, F):
    nx = len(XSPLIT) - 1
    n3 = S // TM
    nb = D // 128
    HP = H_DIM // 2
    QT = (S - QPRE) // n3
    QAL = math.gcd(QPRE, QT)

    HALF = D // 2
    def xcopy(i, si):
        return pltpu.make_async_copy(x_hbm.at[pl.ds(XSPLIT[i], XSPLIT[i + 1] - XSPLIT[i]), :],
                                     x_v.at[pl.ds(XSPLIT[i], XSPLIT[i + 1] - XSPLIT[i]), :], sem.at[si])
    grp = [
        [pltpu.make_async_copy(wqkv_hbm.at[:, pl.ds(D, HALF)], wk_v.at[:, pl.ds(0, HALF)], sem.at[0])],
        [xcopy(0, 1)],
        [pltpu.make_async_copy(wqkv_hbm.at[:, pl.ds(D + HALF, HALF)], wk_v.at[:, pl.ds(HALF, HALF)], sem.at[2]),
         xcopy(1, 2)],
        [xcopy(2, 3), pltpu.make_async_copy(gw_hbm, gw_v, sem.at[3])],
        [xcopy(3, 4),
         pltpu.make_async_copy(wqkv_hbm.at[:, pl.ds(0, D)], wq_v, sem.at[4]),
         pltpu.make_async_copy(wqkv_hbm.at[:, pl.ds(2 * D, D)], wv_v, sem.at[4]),
         pltpu.make_async_copy(wo_hbm, wo_v, sem.at[4])],
        [pltpu.make_async_copy(wg_hbm, wg_v, sem.at[5]),
         pltpu.make_async_copy(wu_hbm, wu_v, sem.at[5]),
         pltpu.make_async_copy(wd_hbm, wd_v, sem.at[5])],
    ]
    for g_ in grp:
        for c in g_:
            c.start()

    def wait(k):
        for c in grp[k]:
            c.wait()

    def q_proj(rows):
        wqp = pltpu.bitcast(wqp_v[...], bf16)
        q = lax.dot_general(x_v[rows, :], wqp, NT, preferred_element_type=f32)
        pq_v[rows, :] = _phi(q)

    def kv_unit(c0, c1, r0, r1):
        xt = x_v[r0:r1, :]
        wkt = pltpu.bitcast(wkt_v[c0 // 2:c1 // 2, :], bf16)
        pkt = _phi(lax.dot_general(wkt, xt, NT, preferred_element_type=f32))
        zs = pkt[:, 0:128]
        for j in range(1, (r1 - r0) // 128):
            zs = zs + pkt[:, j * 128:(j + 1) * 128]
        pp = jnp.dot(pkt.astype(bf16), xt, preferred_element_type=f32)
        if r0 == 0:
            p_v[c0:c1, :] = pp
            z_v[c0:c1, :] = zs
        else:
            p_v[c0:c1, :] += pp
            z_v[c0:c1, :] += zs

    def gate(r0, r1):
        gw = gw_v[...].astype(f32).reshape(1, D)
        g = _sigmoid(jnp.sum(x_v[r0:r1, :].astype(f32) * gw, axis=1, keepdims=True))
        g_v[r0:r1, :] = jnp.broadcast_to(g, (r1 - r0, 128))

    def prologue():
        wait(0)
        wkt_v[0:HALF // 2, :] = pltpu.bitcast(wk_v[:, 0:HALF].T, u32)
        wait(1)
        kv_unit(0, HALF, XSPLIT[0], XSPLIT[1])
        wait(2)
        wkt_v[HALF // 2:D // 2, :] = pltpu.bitcast(wk_v[:, HALF:D].T, u32)
        kv_unit(0, HALF, XSPLIT[1], XSPLIT[2])
        kv_unit(HALF, D, XSPLIT[0], XSPLIT[2])
        wait(3)
        if GSPLIT > 0 and GPOS == 0:
            gate(0, GSPLIT)
        for r0 in range(XSPLIT[2], XSPLIT[3], SUB1):
            kv_unit(0, D, r0, r0 + SUB1)
        wait(4)
        if GSPLIT < GSPLIT2 and GPOS == 0:
            gate(GSPLIT, GSPLIT2)
        for j in range(nb):
            wqt_v[j] = pltpu.bitcast(wq_v[j * 128:(j + 1) * 128, :].T, u32)
        for e in range(HP):
            for j in range(nb):
                wqp_v[e * N_HEADS:(e + 1) * N_HEADS, j * 128:(j + 1) * 128] = (
                    wqt_v[j, pl.ds(e, N_HEADS, stride=HP), :])
        for n, r0 in enumerate(range(XSPLIT[3], XSPLIT[4], SUB1)):
            if n == QEARLY_POS and QEARLY > 0:
                q_proj(pl.ds(0, QEARLY))
            kv_unit(0, D, r0, r0 + SUB1)
        if GSPLIT2 < S and GPOS == 0:
            gate(GSPLIT2, S)

        r = lax.broadcasted_iota(jnp.int32, (128, 128), 0) // H_DIM
        c = lax.broadcasted_iota(jnp.int32, (128, 128), 1) // H_DIM
        mask = r == c
        hb = 128 // H_DIM
        for b in range(nb):
            sl = slice(b * 128, (b + 1) * 128)
            pb = p_v[sl, :].astype(bf16)
            kv = jnp.dot(pb, wv_v[:, sl], preferred_element_type=f32)
            kv_v[b] = pltpu.bitcast(jnp.where(mask, kv, 0.0).astype(bf16), u32)
        q_proj(pl.ds(QEARLY, QPRE - QEARLY))
        for b in range(nb):
            sl = slice(b * 128, (b + 1) * 128)
            kvp = jnp.concatenate([kv_v[b, pl.ds(e, hb, stride=HP), :] for e in range(HP)], axis=0)
            mb = jnp.dot(pltpu.bitcast(kvp, bf16), wo_v[sl, :], preferred_element_type=f32)
            mb = pltpu.bitcast(mb.astype(bf16), u32)
            for e in range(HP):
                mp_v[e * N_HEADS + b * hb:e * N_HEADS + (b + 1) * hb, :] = mb[e * hb:(e + 1) * hb, :]
        for d in range(H_DIM):
            zp_v[pl.ds((d // 2) * 2 * N_HEADS + d % 2, N_HEADS, stride=2), :] = z_v[pl.ds(d, N_HEADS, stride=H_DIM), :]
        zrow_v[...] = jnp.broadcast_to(jnp.sum(zp_v[...].T, axis=0, keepdims=True), (8, D))

        wait(5)

    def body(i, carry):
        row = pl.multiple_of(i * TM, TM)
        xt = x_v[pl.ds(row, TM), :]

        def attn():
            zrow = zrow_v[0:1, :]
            pq = pq_v[pl.ds(row, TM), :]
            t = pq * zrow
            u = t[:, 0:128]
            for j in range(1, nb):
                u = u + t[:, j * 128:(j + 1) * 128]
            u = u + pltpu.roll(u, 64, 1)
            lane = lax.broadcasted_iota(jnp.int32, (TM, 128), 1)
            u = u + jnp.where(lane % 2 == 0, pltpu.roll(u, 127, 1), pltpu.roll(u, 1, 1))
            den = u + 1e-6
            rr = g_v[pl.ds(row, TM), :] * pl.reciprocal(den, approx=True)
            w = (pq * jnp.concatenate([rr] * nb, axis=1)).astype(bf16)
            return jnp.dot(w, pltpu.bitcast(mp_v[...], bf16), preferred_element_type=f32)

        acc = None
        a = None
        for cidx in range(F // FC + 1):
            if cidx == QPOS:
                q_proj(pl.ds(pl.multiple_of(QPRE + i * QT, QAL), QT))
            if GPOS > 0 and cidx == GPOS:
                gw = gw_v[...].astype(f32).reshape(1, D)
                g = _sigmoid(jnp.sum(xt.astype(f32) * gw, axis=1, keepdims=True))
                g_v[pl.ds(row, TM), :] = jnp.broadcast_to(g, (TM, 128))
            if cidx == APOS:
                a = attn()
            if cidx == F // FC:
                break
            sl = slice(cidx * FC, (cidx + 1) * FC)
            gg = jnp.dot(xt, wg_v[:, sl], preferred_element_type=f32)
            uu = jnp.dot(xt, wu_v[:, sl], preferred_element_type=f32)
            if SILU == 0:
                h = (gg * _sigmoid(gg) * uu).astype(bf16)
            else:
                hg = 0.5 * gg
                h = ((hg + hg * jnp.tanh(hg)) * uu).astype(bf16)
            d = jnp.dot(h, wd_v[sl, :], preferred_element_type=f32)
            acc = d if acc is None else acc + d
        omg = 1.0 - g_v[pl.ds(row, TM), :]
        out = (a + jnp.concatenate([omg] * nb, axis=1) * acc).astype(o_v.dtype)
        for cb in range(D // 256):
            for rs in range(TM // ORS):
                rows = pl.ds(pl.multiple_of(row + rs * ORS, ORS), ORS)
                cols = pl.ds(cb * 256, 256)
                o_v[rows, cols] = out[rs * ORS:(rs + 1) * ORS, cb * 256:(cb + 1) * 256]
                pltpu.make_async_copy(o_v.at[rows, cols], o_hbm.at[rows, cols], sem.at[0]).start()
        return carry

    def body_u(i, carry):
        pl.when(i == 0)(prologue)
        for k in range(UNR):
            body(i * UNR + k, carry)
        return carry

    lax.fori_loop(0, n3 // UNR, body_u, 0)
    pltpu.make_async_copy(o_v, o_hbm, sem.at[0]).wait()


@jax.jit
def pallas_gated_mix__linear_attn_block__swiglu_ffn__prompt_kernel(
    A_x, A_wqkv, A_wo, B_x, B_w_gate, B_w_up, B_w_down, gate_w):
    B, S, D = A_x.shape
    F = B_w_gate.shape[1]
    x2 = A_x.reshape(S, D)
    any_spec = pl.BlockSpec(memory_space=pl.ANY)
    out = pl.pallas_call(
        functools.partial(_kernel, S=S, D=D, F=F),
        out_shape=jax.ShapeDtypeStruct((S, D), A_x.dtype),
        in_specs=[any_spec] * 7,
        out_specs=any_spec,
        scratch_shapes=[
            pltpu.VMEM((S, D), bf16),
            pltpu.VMEM((D, D), bf16),
            pltpu.VMEM((D, D), bf16),
            pltpu.VMEM((D, D), bf16),
            pltpu.VMEM((D, D), bf16),
            pltpu.VMEM((D, F), bf16),
            pltpu.VMEM((D, F), bf16),
            pltpu.VMEM((F, D), bf16),
            pltpu.VMEM((D,), bf16),
            pltpu.VMEM((S, D), bf16),
            pltpu.VMEM((D // 2, D), u32),
            pltpu.VMEM((D // 128, D // 2, 128), u32),
            pltpu.VMEM((D // 2, D), u32),
            pltpu.VMEM((D, D), f32),
            pltpu.VMEM((D, 128), f32),
            pltpu.VMEM((D, 128), f32),
            pltpu.VMEM((8, D), f32),
            pltpu.VMEM((D // 128, 64, 128), u32),
            pltpu.VMEM((D // 2, D), u32),
            pltpu.VMEM((S, D), f32),
            pltpu.VMEM((S, 128), f32),
            pltpu.SemaphoreType.DMA((6,)),
        ],
        compiler_params=pltpu.CompilerParams(vmem_limit_bytes=100 * 1024 * 1024, disable_bounds_checks=NOBC),
    )(x2, A_wqkv, A_wo, B_w_gate, B_w_up, B_w_down, gate_w)
    return out.reshape(B, S, D)
```

```python
import functools
import math

import jax
import jax.numpy as jnp
from jax import lax
import jax.experimental.pallas as pl
import jax.experimental.pallas.tpu as pltpu

N_HEADS = 32
LANES = 128
XSPLIT = (0, 128, 256, 896, 2048)
TM = 512
UNROLL = 2
FC = 896
QPRE = 512
OPIECES = ((512,), (512,), (256, 256), (128, 128, 128, 64, 32, 32))
N_SEMS = 3

f32 = jnp.float32
bf16 = jnp.bfloat16
u32 = jnp.uint32
NT = (((1,), (1,)), ((), ()))
LOG2E = 1.4426950408889634


def _phi(t):
    return jnp.where(t > 0, t + 1.0, jnp.exp(t)) + 1e-6


def _one_plus_exp_neg(t):
    return 1.0 + jnp.exp2(t * (-LOG2E))


def _sigmoid(t):
    return pl.reciprocal(_one_plus_exp_neg(t), approx=True)


def _sum_lane_blocks(t):
    s = t[:, 0:LANES]
    for j in range(1, t.shape[1] // LANES):
        s = s + t[:, j * LANES:(j + 1) * LANES]
    return s


def _kernel(x_hbm, wqkv_hbm, wo_hbm, wg_hbm, wu_hbm, wd_hbm, gw_hbm, o_hbm,
            x_v, wq_v, wk_v, wv_v, wo_v, wg_v, wu_v, wd_v, gw_v, o_v,
            wkt_v, wqt_v, wqp_v, p_v, z_v, zp_v, zrow_v, kv_v, mp_v, pq_v, gl_v, sem, *, S, D, F):
    n_tiles = S // TM
    nb = D // LANES
    hd = D // N_HEADS
    hp = hd // 2
    hb = LANES // hd
    qt = (S - QPRE) // n_tiles
    half = D // 2

    def x_rows(i):
        rows = pl.ds(XSPLIT[i], XSPLIT[i + 1] - XSPLIT[i])
        return x_hbm.at[rows, :], x_v.at[rows, :]

    def wk_cols(c0, c1):
        return wqkv_hbm.at[:, pl.ds(D + c0, c1 - c0)], wk_v.at[:, pl.ds(c0, c1 - c0)]

    groups = [
        [wk_cols(LANES, half)],
        [wk_cols(0, LANES), x_rows(0)],
        [wk_cols(half, D), x_rows(1)],
        [x_rows(2)],
        [x_rows(3), (wqkv_hbm.at[:, pl.ds(0, D)], wq_v), (wqkv_hbm.at[:, pl.ds(2 * D, D)], wv_v), (wo_hbm, wo_v)],
        [(gw_hbm, gw_v), (wg_hbm, wg_v), (wu_hbm, wu_v), (wd_hbm, wd_v)],
    ]

    def copies(k):
        return [pltpu.make_async_copy(src, dst, sem.at[k % N_SEMS]) for src, dst in groups[k]]

    def wait_group(k):
        for c in copies(k):
            c.wait()
        if k + N_SEMS < len(groups):
            for c in copies(k + N_SEMS):
                c.start()

    for k in range(N_SEMS):
        for c in copies(k):
            c.start()

    def wk_transpose(c0, c1):
        wkt_v[c0 // 2:c1 // 2, :] = pltpu.bitcast(wk_v[:, c0:c1].T, u32)

    def kv_unit(c0, c1, r0, r1, defer=0):
        wkt = pltpu.bitcast(wkt_v[c0 // 2:c1 // 2, :], bf16)
        pkt = _phi(lax.dot_general(wkt, x_v[r0:r1, :], NT, preferred_element_type=f32))
        zs = _sum_lane_blocks(pkt)
        if r0 == 0:
            z_v[c0:c1, :] = zs
        else:
            z_v[c0:c1, :] += zs
        pkb = pkt.astype(bf16)

        def p_update(m0, m1):
            pp = jnp.dot(pkb[m0 - c0:m1 - c0, :], x_v[r0:r1, :], preferred_element_type=f32)
            if r0 == 0:
                p_v[m0:m1, :] = pp
            else:
                p_v[m0:m1, :] += pp

        p_update(c0, c1 - defer)
        return functools.partial(p_update, c1 - defer, c1)

    def q_proj(rows):
        wqp = pltpu.bitcast(wqp_v[...], bf16)
        q = lax.dot_general(x_v[rows, :], wqp, NT, preferred_element_type=f32)
        pq_v[rows, :] = _phi(q)

    def prologue():
        wait_group(0)
        wk_transpose(LANES, half)
        wait_group(1)
        wk_transpose(0, LANES)
        kv_unit(0, half, XSPLIT[0], XSPLIT[1])
        wait_group(2)
        wk_transpose(half, D)
        kv_unit(0, half, XSPLIT[1], XSPLIT[2])
        rest = kv_unit(half, D, XSPLIT[0], XSPLIT[2], defer=64)
        wait_group(3)
        rest()
        kv_unit(0, D, XSPLIT[2], XSPLIT[3] - LANES)
        rest = kv_unit(0, D, XSPLIT[3] - LANES, XSPLIT[3], defer=96)
        wait_group(4)
        rest()
        for j in range(nb):
            wqt_v[j, 0:D // 2, :] = pltpu.bitcast(wq_v[j * LANES:(j + 1) * LANES, :].T, u32)
        for e in range(hp):
            for j in range(nb):
                wqp_v[e * N_HEADS:(e + 1) * N_HEADS, j * LANES:(j + 1) * LANES] = (
                    wqt_v[j, pl.ds(e, N_HEADS, stride=hp), :])
        kv_unit(0, D, XSPLIT[3], XSPLIT[4])

        q_proj(pl.ds(0, QPRE // 2))
        same_head = (lax.broadcasted_iota(jnp.int32, (LANES, LANES), 0) // hd
                     == lax.broadcasted_iota(jnp.int32, (LANES, LANES), 1) // hd)
        for b in range(nb):
            blk = slice(b * LANES, (b + 1) * LANES)
            kv = jnp.dot(p_v[blk, :].astype(bf16), wv_v[:, blk], preferred_element_type=f32)
            kv_v[b, 0:LANES // 2, :] = pltpu.bitcast(jnp.where(same_head, kv, 0.0).astype(bf16), u32)
        q_proj(pl.ds(QPRE // 2, QPRE // 2))
        for b in range(nb):
            kvp = jnp.concatenate([kv_v[b, pl.ds(e, hb, stride=hp), :] for e in range(hp)], axis=0)
            mb = jnp.dot(pltpu.bitcast(kvp, bf16), wo_v[b * LANES:(b + 1) * LANES, :], preferred_element_type=f32)
            for j in range(nb):
                mj = pltpu.bitcast(mb[:, j * LANES:(j + 1) * LANES].astype(bf16), u32)
                for e in range(hp):
                    m0 = e * N_HEADS + b * hb
                    mp_v[m0:m0 + hb, j * LANES:(j + 1) * LANES] = mj[e * hb:(e + 1) * hb, :]
        for d in range(hd):
            zp_v[pl.ds((d // 2) * 2 * N_HEADS + d % 2, N_HEADS, stride=2), :] = (
                z_v[pl.ds(d, N_HEADS, stride=hd), :])
        zrow_v[...] = jnp.broadcast_to(jnp.sum(zp_v[0:D, :].T, axis=0, keepdims=True), zrow_v.shape)
        wait_group(5)

    def tile(i):
        row = pl.multiple_of(i * TM, TM)
        rows = pl.ds(row, TM)
        xt = x_v[rows, :]

        def ffn_chunk(c):
            cols = slice(c * FC, (c + 1) * FC)
            gg = jnp.dot(xt, wg_v[:, cols], preferred_element_type=f32)
            uu = jnp.dot(xt, wu_v[:, cols], preferred_element_type=f32)
            h = (gg * _sigmoid(gg) * uu).astype(bf16)
            return jnp.dot(h, wd_v[cols, :], preferred_element_type=f32)

        ffn = ffn_chunk(0)
        q_proj(pl.ds(pl.multiple_of(QPRE + i * qt, math.gcd(QPRE, qt)), qt))
        gw = gw_v[...].astype(f32).reshape(1, D)
        gl_v[rows, :] = jnp.broadcast_to(jnp.sum(xt.astype(f32) * gw, axis=1, keepdims=True), (TM, LANES))
        for c in range(1, F // FC):
            ffn = ffn + ffn_chunk(c)

        pq = pq_v[rows, :]
        u = _sum_lane_blocks(pq * zrow_v[0:1, :])
        u = u + pltpu.roll(u, LANES // 2, 1)
        even = lax.broadcasted_iota(jnp.int32, (TM, LANES), 1) % 2 == 0
        den = u + jnp.where(even, pltpu.roll(u, LANES - 1, 1), pltpu.roll(u, 1, 1)) + 1e-6
        g_over_den = pl.reciprocal(den * _one_plus_exp_neg(gl_v[rows, :]), approx=True)
        w = (pq * jnp.concatenate([g_over_den] * nb, axis=1)).astype(bf16)
        ga = jnp.dot(w, pltpu.bitcast(mp_v[...], bf16), preferred_element_type=f32)

        one_minus_g = _sigmoid(-gl_v[rows, :])
        for j in range(nb):
            blk = slice(j * LANES, (j + 1) * LANES)
            out = (ga[:, blk] + one_minus_g * ffn[:, blk]).astype(o_v.dtype)
            r0 = 0
            for n in OPIECES[j]:
                piece = (pl.ds(pl.multiple_of(row + r0, 32), n), pl.ds(j * LANES, LANES))
                o_v[piece] = out[r0:r0 + n, :]
                pltpu.make_async_copy(o_v.at[piece], o_hbm.at[piece], sem.at[0]).start()
                r0 += n

    def step(i, carry):
        pl.when(i == 0)(prologue)
        for k in range(UNROLL):
            tile(i * UNROLL + k)
        return carry

    lax.fori_loop(0, n_tiles // UNROLL, step, 0)
    pltpu.make_async_copy(o_v, o_hbm, sem.at[0]).wait()


@jax.jit
def pallas_gated_mix__linear_attn_block__swiglu_ffn__prompt_kernel(
    A_x: jax.Array,
    A_wqkv: jax.Array,
    A_wo: jax.Array,
    B_x: jax.Array,
    B_w_gate: jax.Array,
    B_w_up: jax.Array,
    B_w_down: jax.Array,
    gate_w: jax.Array,
):
    del B_x
    B, S, D = A_x.shape
    F = B_w_gate.shape[1]
    assert B == 1 and S == XSPLIT[-1] and D == 4 * LANES and F % FC == 0
    hbm = pl.BlockSpec(memory_space=pl.ANY)
    nb = D // LANES
    out = pl.pallas_call(
        functools.partial(_kernel, S=S, D=D, F=F),
        out_shape=jax.ShapeDtypeStruct((S, D), A_x.dtype),
        in_specs=[hbm] * 7,
        out_specs=hbm,
        scratch_shapes=[
            pltpu.VMEM((S, D), bf16),
            pltpu.VMEM((D, D), bf16),
            pltpu.VMEM((D, D), bf16),
            pltpu.VMEM((D, D), bf16),
            pltpu.VMEM((D, D), bf16),
            pltpu.VMEM((D, F), bf16),
            pltpu.VMEM((D, F), bf16),
            pltpu.VMEM((F, D), bf16),
            pltpu.VMEM((D,), bf16),
            pltpu.VMEM((S, D), bf16),
            pltpu.VMEM((D // 2, D), u32),
            pltpu.VMEM((nb, D // 2 + 8, LANES), u32),
            pltpu.VMEM((D // 2, D), u32),
            pltpu.VMEM((D, D), f32),
            pltpu.VMEM((D + 16, LANES), f32),
            pltpu.VMEM((D + 8, LANES), f32),
            pltpu.VMEM((8, D), f32),
            pltpu.VMEM((nb, LANES // 2 + 8, LANES), u32),
            pltpu.VMEM((D // 2, D), u32),
            pltpu.VMEM((S, D), f32),
            pltpu.VMEM((S, LANES), f32),
            pltpu.SemaphoreType.DMA((N_SEMS,)),
        ],
        compiler_params=pltpu.CompilerParams(
            vmem_limit_bytes=64 * 1024 * 1024, disable_bounds_checks=True),
    )(A_x.reshape(S, D), A_wqkv, A_wo, B_w_gate, B_w_up, B_w_down, gate_w)
    return out.reshape(B, S, D)
```

```python
import functools
import math

import jax
import jax.numpy as jnp
from jax import lax
import jax.experimental.pallas as pl
import jax.experimental.pallas.tpu as pltpu

N_HEADS = 32
LANES = 128
XSPLIT = (0, 128, 256, 896, 2048)
TM = 512
UNROLL = 2
FC = 896
QPRE = 512
OPIECES = ((512,), (512,), (256, 256), (128, 128, 128, 64, 32, 32))
N_SEMS = 3

f32 = jnp.float32
bf16 = jnp.bfloat16
u32 = jnp.uint32
NT = (((1,), (1,)), ((), ()))
LOG2E = 1.4426950408889634


def _phi(t):
    return jnp.where(t > 0, t + 1.0, jnp.exp(t)) + 1e-6


def _one_plus_exp_neg(t):
    return 1.0 + jnp.exp2(t * (-LOG2E))


def _sigmoid(t):
    return pl.reciprocal(_one_plus_exp_neg(t), approx=True)


def _sum_lane_blocks(t):
    s = t[:, 0:LANES]
    for j in range(1, t.shape[1] // LANES):
        s = s + t[:, j * LANES:(j + 1) * LANES]
    return s


def _kernel(x_hbm, wqkv_hbm, wo_hbm, wg_hbm, wu_hbm, wd_hbm, gw_hbm, o_hbm,
            x_v, wq_v, wk_v, wv_v, wo_v, wg_v, wu_v, wd_v, gw_v, o_v,
            wkt_v, wqt_v, wqp_v, p_v, z_v, zrow_v, kv_v, mp_v, pq_v, gl_v, sem, *, S, D, F):
    n_tiles = S // TM
    nb = D // LANES
    hd = D // N_HEADS
    hp = hd // 2
    hb = LANES // hd
    qt = (S - QPRE) // n_tiles
    half = D // 2

    def x_rows(i):
        rows = pl.ds(XSPLIT[i], XSPLIT[i + 1] - XSPLIT[i])
        return x_hbm.at[rows, :], x_v.at[rows, :]

    def wk_cols(c0, c1):
        return wqkv_hbm.at[:, pl.ds(D + c0, c1 - c0)], wk_v.at[:, pl.ds(c0, c1 - c0)]

    groups = [
        [wk_cols(LANES, half)],
        [wk_cols(0, LANES), x_rows(0)],
        [wk_cols(half, D), x_rows(1)],
        [x_rows(2)],
        [x_rows(3), (wqkv_hbm.at[:, pl.ds(0, D)], wq_v), (wqkv_hbm.at[:, pl.ds(2 * D, D)], wv_v), (wo_hbm, wo_v)],
        [(gw_hbm, gw_v), (wg_hbm, wg_v), (wu_hbm, wu_v), (wd_hbm, wd_v)],
    ]

    def copies(k):
        return [pltpu.make_async_copy(src, dst, sem.at[k % N_SEMS]) for src, dst in groups[k]]

    def wait_group(k):
        for c in copies(k):
            c.wait()
        if k + N_SEMS < len(groups):
            for c in copies(k + N_SEMS):
                c.start()

    for k in range(N_SEMS):
        for c in copies(k):
            c.start()

    def wk_transpose(c0, c1):
        wkt_v[c0 // 2:c1 // 2, :] = pltpu.bitcast(wk_v[:, c0:c1].T, u32)

    def kv_unit(c0, c1, r0, r1, defer=0):
        wkt = pltpu.bitcast(wkt_v[c0 // 2:c1 // 2, :], bf16)
        pkt = _phi(lax.dot_general(wkt, x_v[r0:r1, :], NT, preferred_element_type=f32))
        zs = _sum_lane_blocks(pkt)
        if r0 == 0:
            z_v[c0:c1, :] = zs
        else:
            z_v[c0:c1, :] += zs
        pkb = pkt.astype(bf16)

        def p_update(m0, m1):
            pp = jnp.dot(pkb[m0 - c0:m1 - c0, :], x_v[r0:r1, :], preferred_element_type=f32)
            if r0 == 0:
                p_v[m0:m1, :] = pp
            else:
                p_v[m0:m1, :] += pp

        p_update(c0, c1 - defer)
        return functools.partial(p_update, c1 - defer, c1)

    def q_proj(rows):
        wqp = pltpu.bitcast(wqp_v[...], bf16)
        q = lax.dot_general(x_v[rows, :], wqp, NT, preferred_element_type=f32)
        pq_v[rows, :] = _phi(q)

    def prologue():
        wait_group(0)
        wk_transpose(LANES, half)
        wait_group(1)
        wk_transpose(0, LANES)
        kv_unit(0, half, XSPLIT[0], XSPLIT[1])
        wait_group(2)
        wk_transpose(half, D)
        kv_unit(0, half, XSPLIT[1], XSPLIT[2])
        rest = kv_unit(half, D, XSPLIT[0], XSPLIT[2], defer=64)
        wait_group(3)
        rest()
        kv_unit(0, D, XSPLIT[2], XSPLIT[3] - LANES)
        rest = kv_unit(0, D, XSPLIT[3] - LANES, XSPLIT[3], defer=96)
        wait_group(4)
        rest()
        for j in range(nb):
            wqt_v[j, 0:D // 2, :] = pltpu.bitcast(wq_v[j * LANES:(j + 1) * LANES, :].T, u32)
        for e in range(hp):
            for j in range(nb):
                wqp_v[e * N_HEADS:(e + 1) * N_HEADS, j * LANES:(j + 1) * LANES] = (
                    wqt_v[j, pl.ds(e, N_HEADS, stride=hp), :])
        kv_unit(0, D, XSPLIT[3], XSPLIT[4])

        q_proj(pl.ds(0, QPRE // 2))
        same_head = (lax.broadcasted_iota(jnp.int32, (LANES, LANES), 0) // hd
                     == lax.broadcasted_iota(jnp.int32, (LANES, LANES), 1) // hd)
        for b in range(nb):
            blk = slice(b * LANES, (b + 1) * LANES)
            kv = jnp.dot(p_v[blk, :].astype(bf16), wv_v[:, blk], preferred_element_type=f32)
            kv_v[b, 0:LANES // 2, :] = pltpu.bitcast(jnp.where(same_head, kv, 0.0).astype(bf16), u32)
        q_proj(pl.ds(QPRE // 2, QPRE // 2))
        for b in range(nb):
            kvp = jnp.concatenate([kv_v[b, pl.ds(e, hb, stride=hp), :] for e in range(hp)], axis=0)
            mb = jnp.dot(pltpu.bitcast(kvp, bf16), wo_v[b * LANES:(b + 1) * LANES, :], preferred_element_type=f32)
            for j in range(nb):
                mj = pltpu.bitcast(mb[:, j * LANES:(j + 1) * LANES].astype(bf16), u32)
                for e in range(hp):
                    m0 = e * N_HEADS + b * hb
                    mp_v[m0:m0 + hb, j * LANES:(j + 1) * LANES] = mj[e * hb:(e + 1) * hb, :]
        znat = jnp.broadcast_to(jnp.sum(z_v[...].T, axis=0, keepdims=True), zrow_v.shape)
        lane = lax.broadcasted_iota(jnp.int32, (zrow_v.shape[0], LANES), 1)
        for j in range(nb):
            src = (lane % (2 * N_HEADS)) // 2 * hd + 2 * (2 * j + lane // (2 * N_HEADS)) + lane % 2
            zj = None
            for b in range(nb):
                got = jnp.take_along_axis(znat[:, b * LANES:(b + 1) * LANES], src % LANES, axis=1)
                zj = got if zj is None else jnp.where(src // LANES == b, got, zj)
            zrow_v[:, j * LANES:(j + 1) * LANES] = zj
        wait_group(5)

    def tile(i):
        row = pl.multiple_of(i * TM, TM)
        rows = pl.ds(row, TM)
        xt = x_v[rows, :]

        def ffn_chunk(c):
            cols = slice(c * FC, (c + 1) * FC)
            gg = jnp.dot(xt, wg_v[:, cols], preferred_element_type=f32)
            uu = jnp.dot(xt, wu_v[:, cols], preferred_element_type=f32)
            h = (gg * _sigmoid(gg) * uu).astype(bf16)
            return jnp.dot(h, wd_v[cols, :], preferred_element_type=f32)

        ffn = ffn_chunk(0)
        q_proj(pl.ds(pl.multiple_of(QPRE + i * qt, math.gcd(QPRE, qt)), qt))
        gw = gw_v[...].astype(f32).reshape(1, D)
        gl_v[rows, :] = jnp.broadcast_to(jnp.sum(xt.astype(f32) * gw, axis=1, keepdims=True), (TM, LANES))
        for c in range(1, F // FC):
            ffn = ffn + ffn_chunk(c)

        pq = pq_v[rows, :]
        u = _sum_lane_blocks(pq * zrow_v[0:1, :])
        u = u + pltpu.roll(u, LANES // 2, 1)
        even = lax.broadcasted_iota(jnp.int32, (TM, LANES), 1) % 2 == 0
        den = u + jnp.where(even, pltpu.roll(u, LANES - 1, 1), pltpu.roll(u, 1, 1)) + 1e-6
        g_over_den = pl.reciprocal(den * _one_plus_exp_neg(gl_v[rows, :]), approx=True)
        w = (pq * jnp.concatenate([g_over_den] * nb, axis=1)).astype(bf16)
        ga = jnp.dot(w, pltpu.bitcast(mp_v[...], bf16), preferred_element_type=f32)

        one_minus_g = _sigmoid(-gl_v[rows, :])
        for j in range(nb):
            blk = slice(j * LANES, (j + 1) * LANES)
            out = (ga[:, blk] + one_minus_g * ffn[:, blk]).astype(o_v.dtype)
            r0 = 0
            for n in OPIECES[j]:
                piece = (pl.ds(pl.multiple_of(row + r0, 32), n), pl.ds(j * LANES, LANES))
                o_v[piece] = out[r0:r0 + n, :]
                pltpu.make_async_copy(o_v.at[piece], o_hbm.at[piece], sem.at[0]).start()
                r0 += n

    def step(i, carry):
        pl.when(i == 0)(prologue)
        for k in range(UNROLL):
            tile(i * UNROLL + k)
        return carry

    lax.fori_loop(0, n_tiles // UNROLL, step, 0)
    pltpu.make_async_copy(o_v, o_hbm, sem.at[0]).wait()


@jax.jit
def pallas_gated_mix__linear_attn_block__swiglu_ffn__prompt_kernel(
    A_x: jax.Array,
    A_wqkv: jax.Array,
    A_wo: jax.Array,
    B_x: jax.Array,
    B_w_gate: jax.Array,
    B_w_up: jax.Array,
    B_w_down: jax.Array,
    gate_w: jax.Array,
):
    del B_x
    B, S, D = A_x.shape
    F = B_w_gate.shape[1]
    assert B == 1 and S == XSPLIT[-1] and D == 4 * LANES and F % FC == 0
    hbm = pl.BlockSpec(memory_space=pl.ANY)
    nb = D // LANES
    out = pl.pallas_call(
        functools.partial(_kernel, S=S, D=D, F=F),
        out_shape=jax.ShapeDtypeStruct((S, D), A_x.dtype),
        in_specs=[hbm] * 7,
        out_specs=hbm,
        scratch_shapes=[
            pltpu.VMEM((S, D), bf16),
            pltpu.VMEM((D, D), bf16),
            pltpu.VMEM((D, D), bf16),
            pltpu.VMEM((D, D), bf16),
            pltpu.VMEM((D, D), bf16),
            pltpu.VMEM((D, F), bf16),
            pltpu.VMEM((D, F), bf16),
            pltpu.VMEM((F, D), bf16),
            pltpu.VMEM((D,), bf16),
            pltpu.VMEM((S, D), bf16),
            pltpu.VMEM((D // 2, D), u32),
            pltpu.VMEM((nb, D // 2 + 8, LANES), u32),
            pltpu.VMEM((D // 2, D), u32),
            pltpu.VMEM((D, D), f32),
            pltpu.VMEM((D, LANES), f32),
            pltpu.VMEM((8, D), f32),
            pltpu.VMEM((nb, LANES // 2 + 8, LANES), u32),
            pltpu.VMEM((D // 2, D), u32),
            pltpu.VMEM((S, D), f32),
            pltpu.VMEM((S, LANES), f32),
            pltpu.SemaphoreType.DMA((N_SEMS,)),
        ],
        compiler_params=pltpu.CompilerParams(
            vmem_limit_bytes=64 * 1024 * 1024, disable_bounds_checks=True),
    )(A_x.reshape(S, D), A_wqkv, A_wo, B_w_gate, B_w_up, B_w_down, gate_w)
    return out.reshape(B, S, D)
```

```python
import functools
import math

import jax
import jax.numpy as jnp
from jax import lax
import jax.experimental.pallas as pl
import jax.experimental.pallas.tpu as pltpu

N_HEADS = 32
LANES = 128
XSPLIT = (0, 128, 256, 896, 2048)
TM = 512
UNROLL = 2
QPRE = 512
CHAINS = 4
OPIECES = ((512,), (512,), (256, 256), (128, 128, 128, 64, 32, 32))
N_SEMS = 3

f32 = jnp.float32
bf16 = jnp.bfloat16
u32 = jnp.uint32
NT = (((1,), (1,)), ((), ()))
LOG2E = 1.4426950408889634


def _phi(t):
    return jnp.where(t > 0, t + 1.0, jnp.exp(t)) + 1e-6


def _one_plus_exp_neg(t):
    return 1.0 + jnp.exp2(t * (-LOG2E))


def _sigmoid(t):
    return pl.reciprocal(_one_plus_exp_neg(t), approx=True)


def _blk(j):
    return slice(j * LANES, (j + 1) * LANES)


def _sum_lane_blocks(t):
    s = t[:, _blk(0)]
    for j in range(1, t.shape[1] // LANES):
        s = s + t[:, _blk(j)]
    return s


def _after(step, dep, val):
    return jnp.where(jnp.full(val.shape, step, jnp.int32) < 0, dep, val)


def _kernel(x_hbm, wqkv_hbm, wo_hbm, wg_hbm, wu_hbm, wd_hbm, gw_hbm, o_hbm,
            x_v, wq_v, wk_v, wv_v, wo_v, wg_v, wu_v, wd_v, gw_v, o_v,
            wkt_v, wqt_v, wqp_v, p_v, z_v, zrow_v, wvt_v, wof_v, m_v, pq_v, gl_v, sem, *, S, D):
    n_tiles = S // TM
    nb = D // LANES
    hd = D // N_HEADS
    hp = hd // 2
    qt = (S - QPRE) // n_tiles
    half = D // 2

    def x_rows(i):
        rows = pl.ds(XSPLIT[i], XSPLIT[i + 1] - XSPLIT[i])
        return x_hbm.at[rows, :], x_v.at[rows, :]

    def wk_cols(c0, c1):
        return wqkv_hbm.at[:, pl.ds(D + c0, c1 - c0)], wk_v.at[:, pl.ds(c0, c1 - c0)]

    groups = [
        [wk_cols(LANES, half)],
        [wk_cols(0, LANES), x_rows(0)],
        [wk_cols(half, D), x_rows(1)],
        [x_rows(2)],
        [x_rows(3), (wqkv_hbm.at[:, pl.ds(0, D)], wq_v), (wqkv_hbm.at[:, pl.ds(2 * D, D)], wv_v), (wo_hbm, wo_v)],
        [(gw_hbm, gw_v), (wg_hbm, wg_v), (wu_hbm, wu_v), (wd_hbm, wd_v)],
    ]

    def copies(k):
        return [pltpu.make_async_copy(src, dst, sem.at[k % N_SEMS]) for src, dst in groups[k]]

    def wait_group(k):
        for c in copies(k):
            c.wait()
        if k + N_SEMS < len(groups):
            for c in copies(k + N_SEMS):
                c.start()

    for k in range(N_SEMS):
        for c in copies(k):
            c.start()

    def wk_transpose(c0, c1):
        wkt_v[c0 // 2:c1 // 2, :] = pltpu.bitcast(wk_v[:, c0:c1].T, u32)

    def kv_unit(c0, c1, r0, r1, defer=0):
        wkt = pltpu.bitcast(wkt_v[c0 // 2:c1 // 2, :], bf16)
        pkt = _phi(lax.dot_general(wkt, x_v[r0:r1, :], NT, preferred_element_type=f32))
        zs = _sum_lane_blocks(pkt)
        if r0 == 0:
            z_v[c0:c1, :] = zs
        else:
            z_v[c0:c1, :] += zs
        pkb = pkt.astype(bf16)

        def p_update(m0, m1):
            pp = jnp.dot(pkb[m0 - c0:m1 - c0, :], x_v[r0:r1, :], preferred_element_type=f32)
            if r0 == 0:
                p_v[m0:m1, :] = pp
            else:
                p_v[m0:m1, :] += pp

        p_update(c0, c1 - defer)
        return functools.partial(p_update, c1 - defer, c1)

    def q_proj(rows):
        wqp = pltpu.bitcast(wqp_v[...], bf16)
        q = lax.dot_general(x_v[rows, :], wqp, NT, preferred_element_type=f32)
        pq_v[rows, :] = _phi(q)

    def prologue(step):
        wait_group(0)
        wk_transpose(LANES, half)
        wait_group(1)
        wk_transpose(0, LANES)
        kv_unit(0, half, XSPLIT[0], XSPLIT[1])
        wait_group(2)
        wk_transpose(half, D)
        kv_unit(0, half, XSPLIT[1], XSPLIT[2])
        rest = kv_unit(half, D, XSPLIT[0], XSPLIT[2], defer=64)
        wait_group(3)
        rest()
        kv_unit(0, D, XSPLIT[2], XSPLIT[3] - LANES)
        rest = kv_unit(0, D, XSPLIT[3] - LANES, XSPLIT[3], defer=96)
        wait_group(4)
        rest()
        for j in range(nb):
            wqt_v[j, 0:D // 2, :] = pltpu.bitcast(wq_v[_blk(j), :].T, u32)
        for e in range(hp):
            for j in range(nb):
                wqp_v[e * N_HEADS:(e + 1) * N_HEADS, _blk(j)] = wqt_v[j, pl.ds(e, N_HEADS, stride=hp), :]
        kv_unit(0, D, XSPLIT[3], XSPLIT[4])

        wvt_v[...] = wv_v[...].T.astype(f32)
        for j in range(nb):
            wof_v[:, _blk(j)] = _after(step, p_v[:, _blk(j)], wo_v[:, _blk(j)].astype(f32))
        q_proj(pl.ds(0, QPRE))
        znat = jnp.broadcast_to(jnp.sum(z_v[...].T, axis=0, keepdims=True), zrow_v.shape)
        lane = lax.broadcasted_iota(jnp.int32, (zrow_v.shape[0], LANES), 1)
        for j in range(nb):
            src = (lane % (2 * N_HEADS)) // 2 * hd + 2 * (2 * j + lane // (2 * N_HEADS)) + lane % 2
            zj = None
            for b in range(nb):
                got = jnp.take_along_axis(znat[:, _blk(b)], src % LANES, axis=1)
                zj = got if zj is None else jnp.where(src // LANES == b, got, zj)
            zrow_v[:, _blk(j)] = zj
        wait_group(5)

    def head_products(step):
        prev = [None] * CHAINS
        for h in range(N_HEADS):
            ph = p_v[h * hd:(h + 1) * hd, :]
            acc = [None] * nb
            for r in range(h * hd, (h + 1) * hd):
                t = None
                for j in range(nb):
                    tj = ph[:, _blk(j)] * wvt_v[r:r + 1, _blk(j)]
                    t = tj if t is None else t + tj
                if prev[r % CHAINS] is not None:
                    t = _after(step, prev[r % CHAINS], t)
                kv = jnp.sum(t, axis=1, keepdims=True)
                prev[r % CHAINS] = kv
                for j in range(nb):
                    mj = kv * wof_v[r:r + 1, _blk(j)]
                    acc[j] = mj if acc[j] is None else acc[j] + mj
            for j in range(nb):
                m_v[j, h * hp:(h + 1) * hp, :] = pltpu.bitcast(acc[j].astype(bf16), u32)

    def tile(i):
        row = pl.multiple_of(i * TM, TM)
        rows = pl.ds(row, TM)
        xt = x_v[rows, :]

        gg = jnp.dot(xt, wg_v[...], preferred_element_type=f32)
        uu = jnp.dot(xt, wu_v[...], preferred_element_type=f32)
        hid = (gg * _sigmoid(gg) * uu).astype(bf16)
        ffn_lo = jnp.dot(hid, wd_v[:, 0:half], preferred_element_type=f32)
        q_proj(pl.ds(pl.multiple_of(QPRE + i * qt, math.gcd(QPRE, qt)), qt))
        gw = gw_v[...].astype(f32).reshape(1, D)
        gl_v[rows, :] = jnp.broadcast_to(jnp.sum(xt.astype(f32) * gw, axis=1, keepdims=True), (TM, LANES))
        ffn = jnp.concatenate([ffn_lo, jnp.dot(hid, wd_v[:, half:D], preferred_element_type=f32)], axis=1)

        pq = pq_v[rows, :]
        u = _sum_lane_blocks(pq * zrow_v[0:1, :])
        u = u + pltpu.roll(u, LANES // 2, 1)
        even = lax.broadcasted_iota(jnp.int32, (TM, LANES), 1) % 2 == 0
        den = u + jnp.where(even, pltpu.roll(u, LANES - 1, 1), pltpu.roll(u, 1, 1)) + 1e-6
        g_over_den = pl.reciprocal(den * _one_plus_exp_neg(gl_v[rows, :]), approx=True)
        w = (pq * jnp.concatenate([g_over_den] * nb, axis=1)).astype(bf16)
        mp = jnp.concatenate(
            [jnp.concatenate([m_v[j, pl.ds(e, N_HEADS, stride=hp), :] for j in range(nb)], axis=1)
             for e in range(hp)], axis=0)
        ga = jnp.dot(w, pltpu.bitcast(mp, bf16), preferred_element_type=f32)

        one_minus_g = _sigmoid(-gl_v[rows, :])
        for j in range(nb):
            out = (ga[:, _blk(j)] + one_minus_g * ffn[:, _blk(j)]).astype(o_v.dtype)
            r0 = 0
            for n in OPIECES[j]:
                piece = (pl.ds(pl.multiple_of(row + r0, 32), n), pl.ds(j * LANES, LANES))
                o_v[piece] = out[r0:r0 + n, :]
                pltpu.make_async_copy(o_v.at[piece], o_hbm.at[piece], sem.at[0]).start()
                r0 += n

    def step_fn(step, carry):
        pl.when(step == 0)(functools.partial(prologue, step))
        head_products(step)
        for k in range(UNROLL):
            tile(step * UNROLL + k)
        return carry

    lax.fori_loop(0, n_tiles // UNROLL, step_fn, 0)
    pltpu.make_async_copy(o_v, o_hbm, sem.at[0]).wait()


@jax.jit
def pallas_gated_mix__linear_attn_block__swiglu_ffn__prompt_kernel(
    A_x: jax.Array,
    A_wqkv: jax.Array,
    A_wo: jax.Array,
    B_x: jax.Array,
    B_w_gate: jax.Array,
    B_w_up: jax.Array,
    B_w_down: jax.Array,
    gate_w: jax.Array,
):
    del B_x
    B, S, D = A_x.shape
    F = B_w_gate.shape[1]
    assert B == 1 and S == XSPLIT[-1] and D == 4 * LANES
    hbm = pl.BlockSpec(memory_space=pl.ANY)
    nb = D // LANES
    out = pl.pallas_call(
        functools.partial(_kernel, S=S, D=D),
        out_shape=jax.ShapeDtypeStruct((S, D), A_x.dtype),
        in_specs=[hbm] * 7,
        out_specs=hbm,
        scratch_shapes=[
            pltpu.VMEM((S, D), bf16),
            pltpu.VMEM((D, D), bf16),
            pltpu.VMEM((D, D), bf16),
            pltpu.VMEM((D, D), bf16),
            pltpu.VMEM((D, D), bf16),
            pltpu.VMEM((D, F), bf16),
            pltpu.VMEM((D, F), bf16),
            pltpu.VMEM((F, D), bf16),
            pltpu.VMEM((D,), bf16),
            pltpu.VMEM((S, D), bf16),
            pltpu.VMEM((D // 2, D), u32),
            pltpu.VMEM((nb, D // 2 + 8, LANES), u32),
            pltpu.VMEM((D // 2, D), u32),
            pltpu.VMEM((D, D), f32),
            pltpu.VMEM((D, LANES), f32),
            pltpu.VMEM((8, D), f32),
            pltpu.VMEM((D, D), f32),
            pltpu.VMEM((D, D), f32),
            pltpu.VMEM((nb, D // 2 + 8, LANES), u32),
            pltpu.VMEM((S, D), f32),
            pltpu.VMEM((S, LANES), f32),
            pltpu.SemaphoreType.DMA((N_SEMS,)),
        ],
        compiler_params=pltpu.CompilerParams(
            vmem_limit_bytes=64 * 1024 * 1024, disable_bounds_checks=True),
    )(A_x.reshape(S, D), A_wqkv, A_wo, B_w_gate, B_w_up, B_w_down, gate_w)
    return out.reshape(B, S, D)
```

```python
import functools
import math

import jax
import jax.numpy as jnp
from jax import lax
import jax.experimental.pallas as pl
import jax.experimental.pallas.tpu as pltpu

N_HEADS = 32
LANES = 128
XSPLIT = (0, 128, 256, 896, 2048)
TM = 512
UNROLL = 2
QPRE = 640
CHAINS = 4
OPIECES = ((512,), (512,), (256, 256), (128, 128, 128, 64, 32, 32))
N_SEMS = 3

f32 = jnp.float32
bf16 = jnp.bfloat16
u32 = jnp.uint32
NT = (((1,), (1,)), ((), ()))
LOG2E = 1.4426950408889634


def _phi(t):
    return jnp.where(t > 0, t + 1.0, jnp.exp(t)) + 1e-6


def _one_plus_exp_neg(t):
    return 1.0 + jnp.exp2(t * (-LOG2E))


def _sigmoid(t):
    return pl.reciprocal(_one_plus_exp_neg(t), approx=True)


def _blk(j):
    return slice(j * LANES, (j + 1) * LANES)


def _sum_lane_blocks(t):
    s = t[:, _blk(0)]
    for j in range(1, t.shape[1] // LANES):
        s = s + t[:, _blk(j)]
    return s


def _after(step, dep, val):
    return jnp.where(jnp.full(val.shape, step, jnp.int32) < 0, dep, val)


def _kernel(x_hbm, wqkv_hbm, wo_hbm, wg_hbm, wu_hbm, wd_hbm, gw_hbm, o_hbm,
            x_v, wq_v, wk_v, wv_v, wo_v, wg_v, wu_v, wd_v, gw_v, o_v,
            wkt_v, wqt_v, wqp_v, p_v, z_v, zrow_v, wvt_v, wof_v, m_v, pq_v, gl_v, sem, *, S, D):
    n_tiles = S // TM
    nb = D // LANES
    hd = D // N_HEADS
    hp = hd // 2
    qt = (S - QPRE) // n_tiles
    half = D // 2

    def x_rows(i):
        rows = pl.ds(XSPLIT[i], XSPLIT[i + 1] - XSPLIT[i])
        return x_hbm.at[rows, :], x_v.at[rows, :]

    def wk_cols(c0, c1):
        return wqkv_hbm.at[:, pl.ds(D + c0, c1 - c0)], wk_v.at[:, pl.ds(c0, c1 - c0)]

    groups = [
        [wk_cols(LANES, half)],
        [wk_cols(0, LANES), x_rows(0)],
        [wk_cols(half, D), x_rows(1)],
        [x_rows(2)],
        [x_rows(3), (wqkv_hbm.at[:, pl.ds(0, D)], wq_v), (wqkv_hbm.at[:, pl.ds(2 * D, D)], wv_v), (wo_hbm, wo_v)],
        [(gw_hbm, gw_v), (wg_hbm, wg_v), (wu_hbm, wu_v), (wd_hbm, wd_v)],
    ]

    def copies(k):
        return [pltpu.make_async_copy(src, dst, sem.at[k % N_SEMS]) for src, dst in groups[k]]

    def wait_group(k):
        for c in copies(k):
            c.wait()
        if k + N_SEMS < len(groups):
            for c in copies(k + N_SEMS):
                c.start()

    for k in range(N_SEMS):
        for c in copies(k):
            c.start()

    def wk_transpose(c0, c1):
        wkt_v[c0 // 2:c1 // 2, :] = pltpu.bitcast(wk_v[:, c0:c1].T, u32)

    def kv_unit(c0, c1, r0, r1, defer=0):
        wkt = pltpu.bitcast(wkt_v[c0 // 2:c1 // 2, :], bf16)
        pkt = _phi(lax.dot_general(wkt, x_v[r0:r1, :], NT, preferred_element_type=f32))
        zs = _sum_lane_blocks(pkt)
        if r0 == 0:
            z_v[c0:c1, :] = zs
        else:
            z_v[c0:c1, :] += zs
        pkb = pkt.astype(bf16)

        def p_update(m0, m1):
            pp = jnp.dot(pkb[m0 - c0:m1 - c0, :], x_v[r0:r1, :], preferred_element_type=f32)
            if r0 == 0:
                p_v[m0:m1, :] = pp
            else:
                p_v[m0:m1, :] += pp

        p_update(c0, c1 - defer)
        return functools.partial(p_update, c1 - defer, c1)

    def q_proj(rows):
        wqp = pltpu.bitcast(wqp_v[...], bf16)
        q = lax.dot_general(x_v[rows, :], wqp, NT, preferred_element_type=f32)
        pq_v[rows, :] = _phi(q)

    def prologue(step):
        wait_group(0)
        wk_transpose(LANES, half)
        wait_group(1)
        wk_transpose(0, LANES)
        kv_unit(0, half, XSPLIT[0], XSPLIT[1])
        wait_group(2)
        wk_transpose(half, D)
        kv_unit(0, half, XSPLIT[1], XSPLIT[2])
        rest = kv_unit(half, D, XSPLIT[0], XSPLIT[2], defer=64)
        wait_group(3)
        rest()
        kv_unit(0, D, XSPLIT[2], XSPLIT[3] - LANES)
        rest = kv_unit(0, D, XSPLIT[3] - LANES, XSPLIT[3], defer=96)
        wait_group(4)
        rest()
        for j in range(nb):
            wqt_v[j, 0:D // 2, :] = pltpu.bitcast(wq_v[_blk(j), :].T, u32)
        for e in range(hp):
            for j in range(nb):
                wqp_v[e * N_HEADS:(e + 1) * N_HEADS, _blk(j)] = wqt_v[j, pl.ds(e, N_HEADS, stride=hp), :]
        kv_unit(0, D, XSPLIT[3], XSPLIT[4])

        wvt_v[...] = wv_v[...].T.astype(f32)
        for j in range(nb):
            wof_v[:, _blk(j)] = _after(step, p_v[:, _blk(j)], wo_v[:, _blk(j)].astype(f32))
        q_proj(pl.ds(0, QPRE))
        znat = jnp.broadcast_to(jnp.sum(z_v[...].T, axis=0, keepdims=True), zrow_v.shape)
        lane = lax.broadcasted_iota(jnp.int32, (zrow_v.shape[0], LANES), 1)
        for j in range(nb):
            src = (lane % (2 * N_HEADS)) // 2 * hd + 2 * (2 * j + lane // (2 * N_HEADS)) + lane % 2
            zj = None
            for b in range(nb):
                got = jnp.take_along_axis(znat[:, _blk(b)], src % LANES, axis=1)
                zj = got if zj is None else jnp.where(src // LANES == b, got, zj)
            zrow_v[:, _blk(j)] = zj
        wait_group(5)

    def head_products(step):
        def head(h, prev):
            prev = list(prev)
            ph = p_v[pl.ds(pl.multiple_of(h * hd, hd), hd), :]
            acc = [None] * nb
            for e in range(hd):
                r = pl.ds(h * hd + e, 1)
                t = None
                for j in range(nb):
                    tj = ph[:, _blk(j)] * wvt_v[r, _blk(j)]
                    t = tj if t is None else t + tj
                kv = jnp.sum(_after(step, prev[e % CHAINS], t), axis=1, keepdims=True)
                prev[e % CHAINS] = kv
                for j in range(nb):
                    mj = kv * wof_v[r, _blk(j)]
                    acc[j] = mj if acc[j] is None else acc[j] + mj
            for j in range(nb):
                m_v[j, pl.ds(pl.multiple_of(h * hp, hp), hp), :] = pltpu.bitcast(acc[j].astype(bf16), u32)
            return tuple(prev)

        lax.fori_loop(0, N_HEADS, head, (jnp.zeros((hd, 1), f32),) * CHAINS, unroll=True)

    def tile(i):
        row = pl.multiple_of(i * TM, TM)
        rows = pl.ds(row, TM)
        xt = x_v[rows, :]

        gg = jnp.dot(xt, wg_v[...], preferred_element_type=f32)
        uu = jnp.dot(xt, wu_v[...], preferred_element_type=f32)
        hid = (gg * _sigmoid(gg) * uu).astype(bf16)
        ffn_lo = jnp.dot(hid, wd_v[:, 0:half], preferred_element_type=f32)
        q_proj(pl.ds(pl.multiple_of(QPRE + i * qt, math.gcd(QPRE, qt)), qt))
        gw = gw_v[...].astype(f32).reshape(1, D)
        gl_v[rows, :] = jnp.broadcast_to(jnp.sum(xt.astype(f32) * gw, axis=1, keepdims=True), (TM, LANES))
        ffn = jnp.concatenate([ffn_lo, jnp.dot(hid, wd_v[:, half:D], preferred_element_type=f32)], axis=1)

        pq = pq_v[rows, :]
        u = _sum_lane_blocks(pq * zrow_v[0:1, :])
        u = u + pltpu.roll(u, LANES // 2, 1)
        even = lax.broadcasted_iota(jnp.int32, (TM, LANES), 1) % 2 == 0
        den = u + jnp.where(even, pltpu.roll(u, LANES - 1, 1), pltpu.roll(u, 1, 1)) + 1e-6
        g_over_den = pl.reciprocal(den * _one_plus_exp_neg(gl_v[rows, :]), approx=True)
        w = (pq * jnp.concatenate([g_over_den] * nb, axis=1)).astype(bf16)
        mp = jnp.concatenate(
            [jnp.concatenate([m_v[j, pl.ds(e, N_HEADS, stride=hp), :] for j in range(nb)], axis=1)
             for e in range(hp)], axis=0)
        ga = jnp.dot(w, pltpu.bitcast(mp, bf16), preferred_element_type=f32)

        one_minus_g = _sigmoid(-gl_v[rows, :])
        for j in range(nb):
            out = (ga[:, _blk(j)] + one_minus_g * ffn[:, _blk(j)]).astype(o_v.dtype)
            r0 = 0
            for n in OPIECES[j]:
                piece = (pl.ds(pl.multiple_of(row + r0, 32), n), pl.ds(j * LANES, LANES))
                o_v[piece] = out[r0:r0 + n, :]
                pltpu.make_async_copy(o_v.at[piece], o_hbm.at[piece], sem.at[0]).start()
                r0 += n

    def step_fn(step, carry):
        pl.when(step == 0)(functools.partial(prologue, step))
        head_products(step)
        for k in range(UNROLL):
            tile(step * UNROLL + k)
        return carry

    lax.fori_loop(0, n_tiles // UNROLL, step_fn, 0)
    pltpu.make_async_copy(o_v, o_hbm, sem.at[0]).wait()


@jax.jit
def pallas_gated_mix__linear_attn_block__swiglu_ffn__prompt_kernel(
    A_x: jax.Array,
    A_wqkv: jax.Array,
    A_wo: jax.Array,
    B_x: jax.Array,
    B_w_gate: jax.Array,
    B_w_up: jax.Array,
    B_w_down: jax.Array,
    gate_w: jax.Array,
):
    del B_x
    B, S, D = A_x.shape
    F = B_w_gate.shape[1]
    assert B == 1 and S == XSPLIT[-1] and D == 4 * LANES
    hbm = pl.BlockSpec(memory_space=pl.ANY)
    nb = D // LANES
    out = pl.pallas_call(
        functools.partial(_kernel, S=S, D=D),
        out_shape=jax.ShapeDtypeStruct((S, D), A_x.dtype),
        in_specs=[hbm] * 7,
        out_specs=hbm,
        scratch_shapes=[
            pltpu.VMEM((S, D), bf16),
            pltpu.VMEM((D, D), bf16),
            pltpu.VMEM((D, D), bf16),
            pltpu.VMEM((D, D), bf16),
            pltpu.VMEM((D, D), bf16),
            pltpu.VMEM((D, F), bf16),
            pltpu.VMEM((D, F), bf16),
            pltpu.VMEM((F, D), bf16),
            pltpu.VMEM((D,), bf16),
            pltpu.VMEM((S, D), bf16),
            pltpu.VMEM((D // 2, D), u32),
            pltpu.VMEM((nb, D // 2 + 8, LANES), u32),
            pltpu.VMEM((D // 2, D), u32),
            pltpu.VMEM((D, D), f32),
            pltpu.VMEM((D, LANES), f32),
            pltpu.VMEM((8, D), f32),
            pltpu.VMEM((D, D), f32),
            pltpu.VMEM((D, D), f32),
            pltpu.VMEM((nb, D // 2 + 8, LANES), u32),
            pltpu.VMEM((S, D), f32),
            pltpu.VMEM((S, LANES), f32),
            pltpu.SemaphoreType.DMA((N_SEMS,)),
        ],
        compiler_params=pltpu.CompilerParams(
            vmem_limit_bytes=64 * 1024 * 1024, disable_bounds_checks=True),
    )(A_x.reshape(S, D), A_wqkv, A_wo, B_w_gate, B_w_up, B_w_down, gate_w)
    return out.reshape(B, S, D)
```
